```python
import jax
import jax.numpy as jnp

def _softmax(x, axis=-1):
    return jax.nn.softmax(x, axis=axis)
def _gelu(x):
    return jax.nn.gelu(x, approximate=True)
def _silu(x):
    return jax.nn.silu(x)
def _sigmoid(x):
    return jax.nn.sigmoid(x)
def _layernorm(x, axis=-1, eps=1e-5):
    m = jnp.mean(x, axis=axis, keepdims=True)
    v = jnp.var(x, axis=axis, keepdims=True)
    return (x - m) / jnp.sqrt(v + eps)
def _scatter_add(tgt, idx, src, axis=0):
    return tgt.at[idx].add(src)
def _segment_sum(src, seg, n):
    return jax.ops.segment_sum(src, seg, n)
class _Rng:
    def __init__(self, key):
        self._k = key
    def _next(self):
        self._k, sub = jax.random.split(self._k)
        return sub
    def normal(self, shape):
        return jax.random.normal(self._next(), shape, dtype=jnp.bfloat16)
    def randint(self, lo, hi, shape):
        return jax.random.randint(self._next(), shape, lo, hi, dtype=jnp.int32)
    def uniform(self, shape, lo=0.0, hi=1.0):
        return jax.random.uniform(self._next(), shape, jnp.bfloat16, lo, hi)
    def permutation(self, n):
        return jax.random.permutation(self._next(), n)


kernel_name = 'parallel_sum__ssm_conv_s5__moe_arch_mod__prompt'

def setup_inputs():
    _rng = _Rng(jax.random.key(int.from_bytes(__import__("os").urandom(4), "little")))
    _w = (lambda a: (lambda t: t.astype(jnp.bfloat16) if jnp.issubdtype(t.dtype, jnp.floating) else t)(jnp.asarray(a)))
    def _A_setup():
        B, S, D = 1, 2048, 1024
        P = D
        Lambda_re = -0.5 * jnp.exp((lambda *s: _rng.normal(s) * 0.05)(P))
        Lambda_im = (lambda *s: _rng.normal(s) * 0.05)(P) * 1.0
        B_re = (lambda *s: _rng.normal(s) * 0.05)(P, D) * (D ** -0.5)
        B_im = (lambda *s: _rng.normal(s) * 0.05)(P, D) * (D ** -0.5)
        C_re = (lambda *s: _rng.normal(s) * 0.05)(D, P) * (P ** -0.5)
        C_im = (lambda *s: _rng.normal(s) * 0.05)(D, P) * (P ** -0.5)
        log_dt = (lambda *s: _rng.normal(s) * 0.05)(P) * 0.3 - 2.0
        Dskip = (lambda *s: _rng.normal(s) * 0.05)(D)
        return {
            "x": _w((lambda *s: _rng.normal(s) * 0.05)(B, S, D)),
            "Lambda_re": _w(Lambda_re),
            "Lambda_im": _w(Lambda_im),
            "B_re": _w(B_re),
            "B_im": _w(B_im),
            "C_re": _w(C_re),
            "C_im": _w(C_im),
            "log_dt": _w(log_dt),
            "Dskip": _w(Dskip),
        }
    _A_in = _A_setup()

    def _B_setup():
        B, S, D, F, C = 1, 2048, 1024, 3584, 2
        return {
            "x": _w((lambda *s: _rng.normal(s) * 0.05)(B, S, D)),
            "w_r": _w((lambda *s: _rng.normal(s) * 0.05)(D)),
            "w_gate": _w((lambda *s: _rng.normal(s) * 0.05)(D, F)),
            "w_up": _w((lambda *s: _rng.normal(s) * 0.05)(D, F)),
            "w_down": _w((lambda *s: _rng.normal(s) * 0.05)(F, D)),
        }
    _B_in = _B_setup()

    return {
        "A_x": _A_in["x"],
        "A_Lambda_re": _A_in["Lambda_re"],
        "A_Lambda_im": _A_in["Lambda_im"],
        "A_B_re": _A_in["B_re"],
        "A_B_im": _A_in["B_im"],
        "A_C_re": _A_in["C_re"],
        "A_C_im": _A_in["C_im"],
        "A_log_dt": _A_in["log_dt"],
        "A_Dskip": _A_in["Dskip"],
        "B_x": _B_in["x"],
        "B_w_r": _B_in["w_r"],
        "B_w_gate": _B_in["w_gate"],
        "B_w_up": _B_in["w_up"],
        "B_w_down": _B_in["w_down"],
    }

def reference(A_x, A_Lambda_re, A_Lambda_im, A_B_re, A_B_im, A_C_re, A_C_im, A_log_dt, A_Dskip, B_x, B_w_r, B_w_gate, B_w_up, B_w_down):
    def _A_ref(x, Lambda_re, Lambda_im, B_re, B_im, C_re, C_im, log_dt, Dskip):
        Bsz, L, H = x.shape
        Lam = Lambda_re + 1j * Lambda_im
        Bmat = B_re + 1j * B_im
        Cmat = C_re + 1j * C_im
        dt = jnp.exp(log_dt)
        Lam_bar = jnp.exp(dt * Lam)
        B_bar = ((Lam_bar - 1.0) / Lam)[:, None] * Bmat
        Bu = jnp.einsum("bld,pd->blp", x + 0j, B_bar)
        h = jnp.zeros_like(Bu[:, 0, :])
        hs = []
        for t in range(L):
            h = Lam_bar[None, :] * h + Bu[:, t, :]
            hs.append(h)
        hseq = jnp.stack(hs, 1)
        y = 2.0 * jnp.einsum("blp,dp->bld", hseq, Cmat).real + x * Dskip[None, None, :]
        return y

    def _B_ref(x, w_r, w_gate, w_up, w_down):
        B, S, D = x.shape
        C = 2
        r = x @ w_r
        idx = jnp.argsort(-r, axis=-1)[:, :C]
        idx_e = jnp.repeat(idx.reshape(B, C, 1), D, axis=2)
        x_sel = jnp.take_along_axis(x, idx_e, axis=1)
        g = _silu(x_sel @ w_gate)
        u = x_sel @ w_up
        y = (g * u) @ w_down
        r_sel = _sigmoid(jnp.take_along_axis(r, idx, axis=1))
        y = y * r_sel.reshape(B, C, 1)
        b_off = (jnp.arange(B) * S).reshape(B, 1)
        flat_idx = (idx + b_off).reshape(B * C)
        zero = (x * 0.0).reshape(B * S, D)
        upd = _scatter_add(zero, flat_idx, y.reshape(B * C, D), axis=0)
        return x + upd.reshape(B, S, D)

    x = A_x
    xn = _layernorm(x, axis=-1)
    return x + _A_ref(xn, A_Lambda_re, A_Lambda_im, A_B_re, A_B_im, A_C_re, A_C_im, A_log_dt, A_Dskip) + _B_ref(xn, B_w_r, B_w_gate, B_w_up, B_w_down)
```

```python
import jax
import jax.numpy as jnp
from jax import lax
import jax.experimental.pallas as pl
import jax.experimental.pallas.tpu as pltpu

L, D, P, F = 2048, 1024, 1024, 3584
T = 256
NC = L // T
G = P // 128
FS = 512
NT = (((1,), (1,)), ((), ()))
f32, bf16 = jnp.float32, jnp.bfloat16


def _rb(v):
    return v.astype(bf16).astype(f32)


def _ln(xf):
    m = jnp.mean(xf, axis=-1, keepdims=True)
    c = xf - m
    v = jnp.mean(c * c, axis=-1, keepdims=True)
    s = _rb(jnp.sqrt(_rb(_rb(v) + 1e-5)))
    return _rb(_rb(xf - _rb(m)) / s)


def _body(x_h, lre, lim, ldt, bre_h, bim_h, cre_h, cim_h, dsk, wr, wg_h, wu_h, wd_h,
          o_h,
          xv, bre, bim, cre, cim, wg, wu, wd, base, hb, xn0, xn1,
          ur0, ui0, ur1, ui1, hr, hi, rs, sx, sw, so):
    def rows(k):
        return pl.ds(pl.multiple_of(k * T, T), T)

    xcp = [pltpu.make_async_copy(x_h.at[pl.ds(k * T, T)], xv.at[pl.ds(k * T, T)], sx.at[k])
           for k in range(NC)]
    H = P // 2
    wsrc = [(bre_h.at[pl.ds(0, H)], bre.at[pl.ds(0, H)]), (bre_h.at[pl.ds(H, H)], bre.at[pl.ds(H, H)]),
            (bim_h.at[pl.ds(0, H)], bim.at[pl.ds(0, H)]), (bim_h.at[pl.ds(H, H)], bim.at[pl.ds(H, H)]),
            (cre_h, cre), (cim_h, cim), (wg_h, wg), (wu_h, wu), (wd_h, wd)]
    wcp = [pltpu.make_async_copy(s, d, sw.at[i]) for i, (s, d) in enumerate(wsrc)]
    xcp[0].start()
    for c in wcp[:4]:
        c.start()
    xcp[1].start()

    dt = _rb(jnp.exp(ldt[...].astype(f32)))
    lr, li = lre[...].astype(f32), lim[...].astype(f32)
    mag = jnp.exp(dt * lr)
    ar, ai = mag * jnp.cos(dt * li), mag * jnp.sin(dt * li)
    den = lr * lr + li * li
    cr = 2.0 * ((ar - 1.0) * lr + ai * li) / den
    ci = 2.0 * (ai * lr - (ar - 1.0) * li) / den
    dskv, wrv = dsk[...].astype(f32), wr[...].astype(f32)

    def ln(k, xn_ref):
        xf = xv[rows(k), :].astype(f32)
        xn = _ln(xf)
        xn_ref[...] = xn.astype(bf16)
        base[rows(k), :] = xf + _rb(xn * dskv) + xn
        rs[rows(k), :] = _rb(jnp.sum(xn * wrv, axis=-1, keepdims=True))

    def bmm_piece(xn_ref, w, u, j0, n):
        r = lax.dot_general(xn_ref[...], w[pl.ds(j0 * 128, n * 128), :], NT, preferred_element_type=f32)
        for j in range(n):
            u[pl.ds(j0 + j, T, stride=G), :] = r[:, j * 128:(j + 1) * 128]

    def bmm(xn_ref, ur, ui):
        bmm_piece(xn_ref, bre, ur, 0, G)
        bmm_piece(xn_ref, bim, ui, 0, G)

    def scan(k, ur, ui, carry):
        h, g = carry
        for t in range(T):
            br, bi = ur[pl.ds(t * G, G), :], ui[pl.ds(t * G, G), :]
            pr = cr * br - ci * bi
            pi = cr * bi + ci * br
            h, g = (ar * h + pr) + ai * g, (ar * g - pi) - ai * h
            hr[pl.ds(t * G, G), :] = h
            hi[pl.ds(t * G, G), :] = g
        for j in range(G):
            hb[rows(k), pl.ds(j * 128, 128)] = hr[pl.ds(j, T, stride=G), :].astype(bf16)
            hb[rows(k), pl.ds(P + j * 128, 128)] = hi[pl.ds(j, T, stride=G), :].astype(bf16)
        return h, g

    xcp[0].wait()
    ln(0, xn0)
    for i, (w, u) in enumerate(((bre, ur0), (bre, ur0), (bim, ui0), (bim, ui0))):
        wcp[i].wait()
        if i == 0:
            for c in xcp[2:]:
                c.start()
        if i == 3:
            for c in wcp[4:]:
                c.start()
        bmm_piece(xn0, w, u, (i % 2) * (G // 2), G // 2)
    xcp[1].wait()
    ln(1, xn1)

    def step2(i, carry):
        k = 2 * i + 1
        xcp_w(k + 1)
        bmm(xn1, ur1, ui1)
        carry = scan(k - 1, ur0, ui0, carry)
        ln(k + 1, xn0)
        xcp_w(k + 2)
        bmm(xn0, ur0, ui0)
        carry = scan(k, ur1, ui1, carry)
        ln(k + 2, xn1)
        return carry

    def xcp_w(k):
        pltpu.make_async_copy(x_h.at[rows(k)], xv.at[rows(k)], sx.at[k]).wait()

    z = jnp.zeros((G, 128), f32)
    carry = lax.fori_loop(0, NC // 2 - 1, step2, (z, z))
    bmm(xn1, ur1, ui1)
    carry = scan(NC - 2, ur0, ui0, carry)

    r = rs[...]
    io = lax.broadcasted_iota(jnp.int32, (L, 1), 0)
    m1 = jnp.max(r)
    i1 = jnp.min(jnp.where(r == m1, io, L))
    r2 = jnp.where(io == i1, -jnp.inf, r)
    m2 = jnp.max(r2)
    i2 = jnp.min(jnp.where((r2 == m2) & (io != i1), io, L))
    i1 = jnp.clip(i1, 0, L - 1)
    i2 = jnp.clip(i2, 0, L - 1)

    def pick(i):
        b = pl.multiple_of((i // 16) * 16, 16)
        blk = xv[pl.ds(b, 16), :].astype(f32)
        s = lax.broadcasted_iota(jnp.int32, (16, 1), 0) == i - b
        return jnp.sum(jnp.where(s, blk, 0.0), axis=0, keepdims=True)

    s16 = lax.broadcasted_iota(jnp.int32, (16, 1), 0)
    xs = _ln(jnp.where(s16 == 0, pick(i1), pick(i2))).astype(bf16)
    for c in wcp[4:]:
        c.wait()
    carry = scan(NC - 1, ur1, ui1, carry)
    ym = jnp.zeros((16, D), f32)
    for f in range(F // FS):
        fs = pl.ds(f * FS, FS)
        a = _rb(jnp.dot(xs, wg[:, fs], preferred_element_type=f32))
        u = _rb(jnp.dot(xs, wu[:, fs], preferred_element_type=f32))
        gu = (_rb(a * jax.nn.sigmoid(a)) * u).astype(bf16)
        ym = ym + jnp.dot(gu, wd[fs, :], preferred_element_type=f32)
    gate = _rb(jax.nn.sigmoid(jnp.where(s16 == 0, m1, m2)))
    ym = _rb(_rb(ym) * gate)
    base[pl.ds(i1, 1), :] = base[pl.ds(i1, 1), :] + ym[0:1]
    base[pl.ds(i2, 1), :] = base[pl.ds(i2, 1), :] + ym[1:2]

    def ocp(k):
        return pltpu.make_async_copy(base.at[rows(k)], o_h.at[rows(k)], so.at[k])

    def cstep(k, _):
        y = lax.dot_general(hb[rows(k), pl.ds(0, P)], cre[...], NT, preferred_element_type=f32)
        y = y + lax.dot_general(hb[rows(k), pl.ds(P, P)], cim[...], NT, preferred_element_type=f32)
        base[rows(k), :] = base[rows(k), :] + y
        ocp(k).start()
        return 0

    lax.fori_loop(0, NC, cstep, 0)
    for k in range(NC):
        ocp(k).wait()


@jax.jit
def pallas_parallel_sum__ssm_conv_s5__moe_arch_mod__prompt_kernel(
        A_x, A_Lambda_re, A_Lambda_im, A_B_re, A_B_im, A_C_re, A_C_im, A_log_dt, A_Dskip,
        B_x, B_w_r, B_w_gate, B_w_up, B_w_down):
    hbm = pl.BlockSpec(memory_space=pl.ANY)
    vm = pl.BlockSpec(memory_space=pltpu.VMEM)
    V = pltpu.VMEM
    out = pl.pallas_call(
        _body,
        out_shape=jax.ShapeDtypeStruct((L, D), f32),
        in_specs=[hbm, vm, vm, vm, hbm, hbm, hbm, hbm, vm, vm, hbm, hbm, hbm],
        out_specs=hbm,
        scratch_shapes=[
            V((L, D), bf16), V((P, D), bf16), V((P, D), bf16), V((D, P), bf16), V((D, P), bf16),
            V((D, F), bf16), V((D, F), bf16), V((F, D), bf16),
            V((L, D), f32), V((L, 2 * P), bf16), V((T, D), bf16), V((T, D), bf16),
            V((T * G, 128), f32), V((T * G, 128), f32), V((T * G, 128), f32), V((T * G, 128), f32),
            V((T * G, 128), f32), V((T * G, 128), f32), V((L, 1), f32),
            pltpu.SemaphoreType.DMA((NC,)), pltpu.SemaphoreType.DMA((9,)), pltpu.SemaphoreType.DMA((NC,)),
        ],
        compiler_params=pltpu.CompilerParams(vmem_limit_bytes=100 * 1024 * 1024),
    )(A_x.reshape(L, D), A_Lambda_re.reshape(G, 128), A_Lambda_im.reshape(G, 128),
      A_log_dt.reshape(G, 128), A_B_re, A_B_im, A_C_re, A_C_im,
      A_Dskip.reshape(1, D), B_w_r.reshape(1, D), B_w_gate, B_w_up, B_w_down)
    return out.reshape(1, L, D)
```

```python
import jax
import jax.numpy as jnp
from jax import lax
import jax.experimental.pallas as pl
import jax.experimental.pallas.tpu as pltpu

L, D, P, F = 2048, 1024, 1024, 3584
T = 256
NC = L // T
G = P // 128
NP = 8
FS = 512
NT = (((1,), (1,)), ((), ()))
f32, bf16 = jnp.float32, jnp.bfloat16


def _rb(v):
    return v.astype(bf16).astype(f32)


def _ln(xf):
    m = jnp.mean(xf, axis=-1, keepdims=True)
    c = xf - m
    v = jnp.mean(c * c, axis=-1, keepdims=True)
    s = _rb(jnp.sqrt(_rb(_rb(v) + 1e-5)))
    return _rb(_rb(xf - _rb(m)) / s)


def _body(x_h, lre, lim, ldt, bre_h, bim_h, cre_h, cim_h, dsk, wr, wg_h, wu_h, wd_h,
          o_h,
          xv, bre, bim, cre, cim, wg, wu, wd, base, hb, xn0, xn1,
          ur0, ui0, ur1, ui1, hr, hi, rs, sx, sw, so):
    def rows(k):
        return pl.ds(pl.multiple_of(k * T, T), T)

    xcp = [pltpu.make_async_copy(x_h.at[pl.ds(k * T, T)], xv.at[pl.ds(k * T, T)], sx.at[k])
           for k in range(NC)]
    H = P // 2
    wsrc = [(bre_h.at[pl.ds(0, H)], bre.at[pl.ds(0, H)]), (bre_h.at[pl.ds(H, H)], bre.at[pl.ds(H, H)]),
            (bim_h.at[pl.ds(0, H)], bim.at[pl.ds(0, H)]), (bim_h.at[pl.ds(H, H)], bim.at[pl.ds(H, H)]),
            (cre_h, cre), (cim_h, cim), (wg_h, wg), (wu_h, wu), (wd_h, wd)]
    wcp = [pltpu.make_async_copy(s, d, sw.at[i]) for i, (s, d) in enumerate(wsrc)]
    xcp[0].start()
    for c in wcp[:4]:
        c.start()
    xcp[1].start()

    dt = _rb(jnp.exp(ldt[...].astype(f32)))
    lr, li = lre[...].astype(f32), lim[...].astype(f32)
    mag = jnp.exp(dt * lr)
    ar, ai = mag * jnp.cos(dt * li), mag * jnp.sin(dt * li)
    den = lr * lr + li * li
    cr = 2.0 * ((ar - 1.0) * lr + ai * li) / den
    ci = 2.0 * (ai * lr - (ar - 1.0) * li) / den
    dskv, wrv = dsk[...].astype(f32).reshape(1, D), wr[...].astype(f32).reshape(1, D)

    Q = T // NP

    def sub(k, q):
        return pl.ds(pl.multiple_of(k * T + q * Q, Q), Q)

    def lnq(k, xn_ref, q):
        xf = xv[sub(k, q), :].astype(f32)
        xn = _ln(xf)
        xn_ref[pl.ds(q * Q, Q), :] = xn.astype(bf16)
        base[sub(k, q), :] = xf + _rb(xn * dskv) + xn
        rs[sub(k, q), :] = _rb(jnp.sum(xn * wrv, axis=-1, keepdims=True))

    def ln(k, xn_ref):
        for q in range(NP):
            lnq(k, xn_ref, q)

    def bmm_piece(xn_ref, w, u, j0, n):
        r = lax.dot_general(xn_ref[...], w[pl.ds(j0 * 128, n * 128), :], NT, preferred_element_type=f32)
        for j in range(n):
            u[pl.ds(j0 + j, T, stride=G), :] = r[:, j * 128:(j + 1) * 128]

    def scanq(k, ur, ui, carry, q):
        h, g = carry
        for t in range(q * Q, (q + 1) * Q):
            br, bi = ur[pl.ds(t * G, G), :], ui[pl.ds(t * G, G), :]
            pr = cr * br - ci * bi
            pi = cr * bi + ci * br
            h, g = (ar * h + pr) + ai * g, (ar * g - pi) - ai * h
            hr[pl.ds(t * G, G), :] = h
            hi[pl.ds(t * G, G), :] = g
        for j in range(G):
            hb[sub(k, q), pl.ds(j * 128, 128)] = hr[pl.ds(q * Q * G + j, Q, stride=G), :].astype(bf16)
            hb[sub(k, q), pl.ds(P + j * 128, 128)] = hi[pl.ds(q * Q * G + j, Q, stride=G), :].astype(bf16)
        return h, g

    def step(k, xa, xb, ua, ub, carry, do_ln=True):
        n = 2 * G // NP
        for q in range(NP):
            c = q // (NP // 2)
            bmm_piece(xa, (bre, bim)[c], ua[c], (q % (NP // 2)) * n, n)
            carry = scanq(k - 1, ub[0], ub[1], carry, q)
            if do_ln:
                lnq(k + 1, xb, q)
        return carry

    xcp[0].wait()
    ln(0, xn0)
    for i, (w, u) in enumerate(((bre, ur0), (bre, ur0), (bim, ui0), (bim, ui0))):
        wcp[i].wait()
        if i == 0:
            for c in xcp[2:]:
                c.start()
        if i == 3:
            for c in wcp[4:]:
                c.start()
        bmm_piece(xn0, w, u, (i % 2) * (G // 2), G // 2)
    xcp[1].wait()
    ln(1, xn1)

    def step2(i, carry):
        k = 2 * i + 1
        xcp_w(k + 1)
        carry = step(k, xn1, xn0, (ur1, ui1), (ur0, ui0), carry)
        xcp_w(k + 2)
        carry = step(k + 1, xn0, xn1, (ur0, ui0), (ur1, ui1), carry)
        return carry

    def xcp_w(k):
        pltpu.make_async_copy(x_h.at[rows(k)], xv.at[rows(k)], sx.at[k]).wait()

    z = jnp.zeros((G, 128), f32)
    carry = lax.fori_loop(0, NC // 2 - 1, step2, (z, z))
    carry = step(NC - 1, xn1, xn0, (ur1, ui1), (ur0, ui0), carry, False)

    r = rs[...]
    io = lax.broadcasted_iota(jnp.int32, (L, 1), 0)
    m1 = jnp.max(r)
    i1 = jnp.min(jnp.where(r == m1, io, L))
    r2 = jnp.where(io == i1, -jnp.inf, r)
    m2 = jnp.max(r2)
    i2 = jnp.min(jnp.where((r2 == m2) & (io != i1), io, L))
    i1 = jnp.clip(i1, 0, L - 1)
    i2 = jnp.clip(i2, 0, L - 1)

    def pick(i):
        b = pl.multiple_of((i // 16) * 16, 16)
        blk = xv[pl.ds(b, 16), :].astype(f32)
        s = lax.broadcasted_iota(jnp.int32, (16, 1), 0) == i - b
        return jnp.sum(jnp.where(s, blk, 0.0), axis=0, keepdims=True)

    s16 = lax.broadcasted_iota(jnp.int32, (16, 1), 0)
    xs = _ln(jnp.where(s16 == 0, pick(i1), pick(i2))).astype(bf16)
    for c in wcp[4:]:
        c.wait()
    def ocp(k):
        return pltpu.make_async_copy(base.at[rows(k)], o_h.at[rows(k)], so.at[k])

    def cstep(k, _):
        y = lax.dot_general(hb[rows(k), pl.ds(0, P)], cre[...], NT, preferred_element_type=f32)
        y = y + lax.dot_general(hb[rows(k), pl.ds(P, P)], cim[...], NT, preferred_element_type=f32)
        base[rows(k), :] = base[rows(k), :] + y
        return 0

    cstep(0, 0)
    ym = jnp.zeros((16, D), f32)
    for f in range(F // FS):
        carry = scanq(NC - 1, ur1, ui1, carry, f)
        fs = pl.ds(f * FS, FS)
        a = _rb(jnp.dot(xs, wg[:, fs], preferred_element_type=f32))
        u = _rb(jnp.dot(xs, wu[:, fs], preferred_element_type=f32))
        gu = (_rb(a * jax.nn.sigmoid(a)) * u).astype(bf16)
        ym = ym + jnp.dot(gu, wd[fs, :], preferred_element_type=f32)
    for q in range(F // FS, NP):
        carry = scanq(NC - 1, ur1, ui1, carry, q)
    gate = _rb(jax.nn.sigmoid(jnp.where(s16 == 0, m1, m2)))
    ym = _rb(_rb(ym) * gate)
    base[pl.ds(i1, 1), :] = base[pl.ds(i1, 1), :] + ym[0:1]
    base[pl.ds(i2, 1), :] = base[pl.ds(i2, 1), :] + ym[1:2]

    ocp(0).start()

    @pl.loop(1, NC)
    def _(k):
        cstep(k, 0)
        ocp(k).start()

    for k in range(NC):
        ocp(k).wait()


@jax.jit
def pallas_parallel_sum__ssm_conv_s5__moe_arch_mod__prompt_kernel(
        A_x, A_Lambda_re, A_Lambda_im, A_B_re, A_B_im, A_C_re, A_C_im, A_log_dt, A_Dskip,
        B_x, B_w_r, B_w_gate, B_w_up, B_w_down):
    hbm = pl.BlockSpec(memory_space=pl.ANY)
    vm = pl.BlockSpec(memory_space=pltpu.VMEM)
    V = pltpu.VMEM
    out = pl.pallas_call(
        _body,
        out_shape=jax.ShapeDtypeStruct((L, D), f32),
        in_specs=[hbm, vm, vm, vm, hbm, hbm, hbm, hbm, vm, vm, hbm, hbm, hbm],
        out_specs=hbm,
        scratch_shapes=[
            V((L, D), bf16), V((P, D), bf16), V((P, D), bf16), V((D, P), bf16), V((D, P), bf16),
            V((D, F), bf16), V((D, F), bf16), V((F, D), bf16),
            V((L, D), f32), V((L, 2 * P), bf16), V((T, D), bf16), V((T, D), bf16),
            V((T * G, 128), f32), V((T * G, 128), f32), V((T * G, 128), f32), V((T * G, 128), f32),
            V((T * G, 128), f32), V((T * G, 128), f32), V((L, 1), f32),
            pltpu.SemaphoreType.DMA((NC,)), pltpu.SemaphoreType.DMA((9,)), pltpu.SemaphoreType.DMA((NC,)),
        ],
        compiler_params=pltpu.CompilerParams(flags={'XLA_TPU_EVENLY_DISTRIBUTE_CRITICAL_NODES':True},vmem_limit_bytes=100 * 1024 * 1024),
    )(A_x.reshape(L, D), A_Lambda_re.reshape(G, 128), A_Lambda_im.reshape(G, 128),
      A_log_dt.reshape(G, 128), A_B_re, A_B_im, A_C_re, A_C_im,
      A_Dskip, B_w_r, B_w_gate, B_w_up, B_w_down)
    return out.reshape(1, L, D)
```
